```python
import os as _os
_os.environ.setdefault("JAX_PLATFORMS", "cpu")
import jax
import jax.numpy as jnp

def _softmax(x, axis=-1):
    return jax.nn.softmax(x, axis=axis)
def _gelu(x):
    return jax.nn.gelu(x, approximate=True)
def _silu(x):
    return jax.nn.silu(x)
def _sigmoid(x):
    return jax.nn.sigmoid(x)
def _layernorm(x, axis=-1, eps=1e-5):
    m = jnp.mean(x, axis=axis, keepdims=True)
    v = jnp.var(x, axis=axis, keepdims=True)
    return (x - m) / jnp.sqrt(v + eps)
def _scatter_add(tgt, idx, src, axis=0):
    return tgt.at[idx].add(src)
def _segment_sum(src, seg, n):
    return jax.ops.segment_sum(src, seg, n)
class _Rng:
    def __init__(self, key):
        self._k = key
    def _next(self):
        self._k, sub = jax.random.split(self._k)
        return sub
    def normal(self, shape):
        return jax.random.normal(self._next(), shape, dtype=jnp.bfloat16)
    def randint(self, lo, hi, shape):
        return jax.random.randint(self._next(), shape, lo, hi, dtype=jnp.int32)
    def uniform(self, shape, lo=0.0, hi=1.0):
        return jax.random.uniform(self._next(), shape, jnp.bfloat16, lo, hi)
    def permutation(self, n):
        return jax.random.permutation(self._next(), n)


kernel_name = 'interleave_layers__sliding_local_dilated__glu_gated_reglu__prompt'

def setup_inputs():
    _rng = _Rng(jax.random.key(int.from_bytes(__import__("os").urandom(4), "little")))
    _w = (lambda a: (lambda t: t.astype(jnp.bfloat16) if jnp.issubdtype(t.dtype, jnp.floating) else t)(jnp.asarray(a)))
    def _A_setup():
        B, S, D = 1, 2048, 512
        return {
            "x": _w((lambda *s: _rng.normal(s) * 0.05)(B, S, D)),
            "wqkv": _w((lambda *s: _rng.normal(s) * 0.05)(D, 3 * D)),
            "wo": _w((lambda *s: _rng.normal(s) * 0.05)(D, D)),
        }
    _A_in = _A_setup()

    def _B_setup():
        B, S, D, F = 1, 2048, 512, 1792
        return {
            "x": _w((lambda *s: _rng.normal(s) * 0.05)(B, S, D)),
            "W_gate": _w((lambda *s: _rng.normal(s) * 0.8)(D, F) * (2.0 / D) ** 0.5),
            "W_up": _w((lambda *s: _rng.normal(s) * 0.8)(D, F) * (2.0 / D) ** 0.5),
            "W_down": _w((lambda *s: _rng.normal(s) * 0.8)(F, D) * (1.0 / F) ** 0.5),
        }
    _B_in = _B_setup()

    return {
        "A_x": _A_in["x"],
        "A_wqkv": _A_in["wqkv"],
        "A_wo": _A_in["wo"],
        "B_x": _B_in["x"],
        "B_W_gate": _B_in["W_gate"],
        "B_W_up": _B_in["W_up"],
        "B_W_down": _B_in["W_down"],
    }

def reference(A_x, A_wqkv, A_wo, B_x, B_W_gate, B_W_up, B_W_down):
    def _A_ref(x, wqkv, wo):
        B, S, D = x.shape
        H = 32; Dh = D // H
        W, dil = 8, 2
        qkv = (lambda x, *d: x.transpose(*d))((x @ wqkv).reshape(B, S, 3, H, Dh), 2, 0, 3, 1, 4)
        q, k, v = qkv[0], qkv[1], qkv[2]
        scale = Dh ** -0.5
        pos = jnp.arange(S)
        off = jnp.arange(W) * dil
        idx = pos[:, None] - off[None, :]
        mask = idx >= 0
        idx_c = jnp.where(mask, idx, 0).reshape(-1)
        kg = k[:, :, idx_c, :].reshape(B, H, S, W, Dh)
        vg = v[:, :, idx_c, :].reshape(B, H, S, W, Dh)
        logits = jnp.einsum("bhsd,bhswd->bhsw", q, kg) * scale
        logits = jnp.where(mask[None, None, :, :], logits, -1e9)
        attn = _softmax(logits, axis=-1)
        o = jnp.einsum("bhsw,bhswd->bhsd", attn, vg)
        return (lambda x, *d: x.transpose(*d))(o, 0, 2, 1, 3).reshape(B, S, D) @ wo

    def _B_ref(x, W_gate, W_up, W_down):
        gate = jnp.einsum("bsd,df->bsf", x, W_gate)
        up = jnp.einsum("bsd,df->bsf", x, W_up)
        gate = gate * (lambda x, dt: x.astype(dt))(gate > 0, gate.dtype)
        h = gate * up
        return jnp.einsum("bsf,fd->bsd", h, W_down)

    x = A_x
    x = x + _A_ref(_layernorm(x, axis=-1), A_wqkv, A_wo)
    x = x + _B_ref(_layernorm(x, axis=-1), B_W_gate, B_W_up, B_W_down)
    x = x + _A_ref(_layernorm(x, axis=-1), A_wqkv, A_wo)
    x = x + _B_ref(_layernorm(x, axis=-1), B_W_gate, B_W_up, B_W_down)
    return x
```

```python
import functools
import math

import jax
import jax.numpy as jnp
from jax import lax
from jax.experimental import pallas as pl
from jax.experimental.pallas import tpu as pltpu

F32, BF16 = jnp.float32, jnp.bfloat16
S, D, F = 2048, 512, 1792
LANES = 128
HEADS, DH, WIN, DIL = 32, 16, 8, 2
HALO = 16
LOG2E = math.log2(math.e)


def _quads(b):
    h = len(b) // 2
    return [[[r[j * h:(j + 1) * h] for r in b[i * h:(i + 1) * h]] for j in range(2)] for i in range(2)]


def _ew(f, x, y):
    return [[f(p, q) for p, q in zip(rx, ry)] for rx, ry in zip(x, y)]


_add = functools.partial(_ew, lambda p, q: p + q)
_sub = functools.partial(_ew, lambda p, q: p - q)


def lhs_ops(b):
    if len(b) == 1:
        return [b[0][0]]
    (a11, a12), (a21, a22) = _quads(b)
    ops = [_add(a11, a22), _add(a21, a22), a11, a22, _add(a11, a12), _sub(a21, a11), _sub(a12, a22)]
    return [o for x in ops for o in lhs_ops(x)]


def rhs_ops(b):
    if len(b) == 1:
        return [b[0][0]]
    (b11, b12), (b21, b22) = _quads(b)
    ops = [_add(b11, b22), b11, _sub(b12, b22), _sub(b21, b11), b22, _add(b11, b12), _add(b21, b22)]
    return [o for x in ops for o in rhs_ops(x)]


def combine(prod, lvl, base=0):
    if lvl == 0:
        return [[prod(base)]]
    n = 7 ** (lvl - 1)
    m = lambda i: combine(prod, lvl - 1, base + i * n)
    m1 = m(0)
    m2 = m(1)
    c22 = _sub(m1, m2)
    m4 = m(3)
    c21 = _add(m2, m4)
    c11 = _add(m1, m4)
    m3 = m(2)
    c22 = _add(c22, m3)
    m5 = m(4)
    c12 = _add(m3, m5)
    c11 = _sub(c11, m5)
    c11 = _add(c11, m(6))
    c22 = _add(c22, m(5))
    return [l + r for l, r in zip(c11, c12)] + [l + r for l, r in zip(c21, c22)]


def interleave(*streams):
    items = []
    for s in streams:
        for i, f in enumerate(s):
            items.append(((i + 0.5) / len(s), f))
    items.sort(key=lambda t: t[0])
    for _, f in items:
        f()


def build(T=256, lq=0, lo=0, lg=0, ld=0, ac=16, lc=16, name="fused", only_loop=False):
    NT = S // T
    RQ, RO, RG, RD = 2 ** lq, 2 ** lo, 2 ** lg, 2 ** ld
    GQ, GO, GG, GD = 12 // RQ, 4 // RO, 28 // max(RG, 2), 4 // RD

    def kernel(x_hbm, wqkv_hbm, wo_hbm, wg_hbm, wu_hbm, wd_hbm, o_hbm,
               xin, xout, wqkv_raw, wo_raw, wg_raw, wu_raw, wd_raw, wo_f32,
               wq_p, wo_p, wg_p, wd_p,
               xa_res, xf_res, a_ops, f_ops, o_ops, h_ops, q_buf, k_buf, v_buf,
               sem_x, sem_w, sem_o):
        def x_copy(t):
            return pltpu.make_async_copy(x_hbm.at[pl.ds(t * T, T)], xin.at[t], sem_x.at[t])

        def o_copy(t):
            return pltpu.make_async_copy(xout.at[t], o_hbm.at[pl.ds(pl.multiple_of(t * T, T), T)], sem_o.at[t])

        w_copies = [pltpu.make_async_copy(s, d, sem_w.at[i]) for i, (s, d) in enumerate(
            [(wqkv_hbm, wqkv_raw), (wo_hbm, wo_raw), (wg_hbm, wg_raw), (wu_hbm, wu_raw), (wd_hbm, wd_raw)])]

        def tile(n):
            return slice(n * LANES, (n + 1) * LANES)

        def prep_wqkv():
            lane = lax.broadcasted_iota(jnp.int32, (8, LANES), 1)
            dgrp = (lane >> 2) & 3
            cols = []
            for part in range(3):
                src = [pltpu.bitcast(wqkv_raw[:, tile(4 * part + j)], jnp.int32) for j in range(4)]
                for i in range(4):
                    gf = jnp.broadcast_to(dgrp[:1], src[0].shape)
                    m = jnp.where(gf == i, src[0], jnp.where(gf == (i + 1) % 4, src[1],
                                  jnp.where(gf == (i + 2) % 4, src[2], src[3])))
                    idx = (lane & 7) * 16 + 4 * ((i + ((lane >> 3) & 3)) & 3) + (lane >> 5)
                    idx = jnp.broadcast_to(idx[:1], m.shape)
                    cols.append(pltpu.bitcast(jnp.take_along_axis(m, idx, axis=1), BF16))
            kb = D // RQ
            for g in range(GQ):
                blk = [[cols[g * RQ + j][i * kb:(i + 1) * kb] for j in range(RQ)] for i in range(RQ)]
                if lq:
                    blk = [[b.astype(F32) for b in r] for r in blk]
                for n, op in enumerate(rhs_ops(blk)):
                    wq_p[g * 7 ** lq + n] = op.astype(BF16)

        def prep_wo():
            for c in range(4):
                wo_f32[c] = wo_raw[:, tile(c)].astype(F32)
            cols = []
            for c in range(4):
                rows = []
                for i in range(4):
                    for dd in range(4):
                        for j in range(4):
                            rows.append(wo_f32[c, pl.ds(j * 128 + 4 * ((i + j) % 4) + dd, 8, stride=16), :])
                cols.append(jnp.concatenate(rows, axis=0))
            kb = D // RO
            for g in range(GO):
                blk = [[cols[g * RO + j][i * kb:(i + 1) * kb] for j in range(RO)] for i in range(RO)]
                for n, op in enumerate(rhs_ops(blk)):
                    wo_p[g * 7 ** lo + n] = op.astype(BF16)

        def gu_cols(g):
            if lg == 2:
                return [(wg_raw, g), (wu_raw, g), (wg_raw, g + 7), (wu_raw, g + 7)]
            return [(wg_raw, g), (wu_raw, g)]

        def prep_wg():
            if lg == 0:
                return
            kb = D // RG
            for g in range(GG):
                blk = [[r[i * kb:(i + 1) * kb, tile(c)].astype(F32) for r, c in gu_cols(g)] for i in range(RG)]
                for n, op in enumerate(rhs_ops(blk)):
                    wg_p[g * 7 ** lg + n] = op.astype(BF16)

        def prep_wd():
            if ld == 0:
                return
            kb = F // RD
            for g in range(GD):
                for r0 in range(0, kb, 128):
                    blk = [[wd_raw[i * kb + r0:i * kb + r0 + 128, tile(g * RD + j)].astype(F32)
                            for j in range(RD)] for i in range(RD)]
                    for n, op in enumerate(rhs_ops(blk)):
                        wd_p[g * 7 ** ld + n, r0:r0 + 128, :] = op.astype(BF16)

        def dot(a, b):
            return jnp.dot(a, b, preferred_element_type=F32)

        def norm(x):
            m = jnp.sum(x, axis=-1, keepdims=True) * (1.0 / D)
            d = x - m
            v = jnp.sum(d * d, axis=-1, keepdims=True) * (1.0 / D)
            return d * lax.rsqrt(v + 1e-5)

        def store_ops(dst, rows, r0, nr, R):
            kb = rows[0].shape[1] // R
            blk = [[x[:, j * kb:(j + 1) * kb] for j in range(R)] for x in rows]
            for n, op in enumerate(lhs_ops(blk)):
                dst[n, r0:r0 + nr, :] = op.astype(BF16)

        def ln_a_steps(t, first_layer):
            def step(r0):
                rows = []
                for i in range(RQ):
                    rs = pl.ds(i * (T // RQ) + r0, lc)
                    x = xin[t, rs, :].astype(F32)
                    if first_layer is not True:
                        x = jnp.where(first_layer, x, xa_res[t, rs, :])
                    xa_res[t, rs, :] = x
                    rows.append(norm(x))
                store_ops(a_ops, rows, r0, lc, RQ)
            return [functools.partial(step, r0) for r0 in range(0, T // RQ, lc)]

        def ln_f_steps(slot):
            def step(r0):
                rows = [norm(xf_res[slot, pl.ds(i * (T // RG) + r0, lc), :]) for i in range(RG)]
                store_ops(f_ops, rows, r0, lc, RG)
            return [functools.partial(step, r0) for r0 in range(0, T // RG, lc)]

        def qkv_steps(first_tile):
            m = T // RQ

            def halo():
                for c in range(4):
                    k_buf[c, 0:HALO, :] = k_buf[c, T:T + HALO, :]
                    v_buf[c, 0:HALO, :] = v_buf[c, T:T + HALO, :]

            def step(g):
                out = combine(lambda n: dot(a_ops[n], wq_p[g * 7 ** lq + n]), lq)
                for i in range(RQ):
                    for j in range(RQ):
                        part, c = divmod(g * RQ + j, 4)
                        if part == 0:
                            q_buf[c, i * m:(i + 1) * m, :] = out[i][j] * (DH ** -0.5 * LOG2E)
                        else:
                            (k_buf, v_buf)[part - 1][c, HALO + i * m:HALO + (i + 1) * m, :] = out[i][j]
                        if part == 2 and i == 0:
                            v0 = jnp.broadcast_to(out[0][j][0:1], (HALO, LANES))
                            if first_tile is True:
                                v_buf[c, 0:HALO, :] = v0
                            else:
                                v_buf[c, 0:HALO, :] = jnp.where(first_tile, v0, v_buf[c, 0:HALO, :])
            steps = [functools.partial(step, g) for g in range(GQ)]
            return steps if first_tile is True else [halo] + steps

        def attend(r0, nr, first_tile):
            q = [q_buf[c, r0:r0 + nr, :] for c in range(4)]
            lg_ = []
            for w in range(WIN):
                s = HALO + r0 - DIL * w
                p = (q[0] * k_buf[0, s:s + nr, :] + q[1] * k_buf[1, s:s + nr, :]) + (
                    q[2] * k_buf[2, s:s + nr, :] + q[3] * k_buf[3, s:s + nr, :])
                p = p + pltpu.roll(p, 64, 1)
                p = p + pltpu.roll(p, 32, 1)
                if r0 < DIL * w:
                    row = r0 + lax.broadcasted_iota(jnp.int32, (nr, LANES), 0)
                    lim = DIL * w if first_tile is True else jnp.where(first_tile, DIL * w, 0)
                    p = jnp.where(row < lim, -1e9 * LOG2E, p)
                lg_.append(p)
            mx = functools.reduce(jnp.maximum, lg_)
            e = [jnp.exp2(p - mx) for p in lg_]
            inv = 1.0 / functools.reduce(lambda a, b: a + b, e)
            o = []
            for c in range(4):
                acc = None
                for w in range(WIN):
                    s = HALO + r0 - DIL * w
                    t = e[w] * v_buf[c, s:s + nr, :]
                    acc = t if acc is None else acc + t
                o.append(acc * inv)
            return jnp.concatenate(o, axis=1)

        def attn_steps(first_tile):
            def step(r0):
                rows = [attend(i * (T // RO) + r0, ac, first_tile) for i in range(RO)]
                store_ops(o_ops, rows, r0, ac, RO)
            return [functools.partial(step, r0) for r0 in range(0, T // RO, ac)]

        def wo_steps(t, slot):
            m = T // RO

            def step(g):
                out = combine(lambda n: dot(o_ops[n], wo_p[g * 7 ** lo + n]), lo)
                for i in range(RO):
                    for j in range(RO):
                        rs, cs = pl.ds(i * m, m), tile(g * RO + j)
                        xf_res[slot, rs, cs] = xa_res[t, rs, cs] + out[i][j]
            return [functools.partial(step, g) for g in range(GO)]

        def gu_steps():
            def hidden(g):
                if lg == 0:
                    out = [[dot(f_ops[0], r[:, tile(c)]) for r, c in gu_cols(g)]]
                else:
                    out = combine(lambda n: dot(f_ops[n], wg_p[g * 7 ** lg + n]), lg)
                return [jnp.concatenate([jnp.maximum(r[j], 0.0) * r[j + 1] for r in out], axis=0)
                        for j in range(0, len(out[0]), 2)]

            def step(g):
                h = hidden(g) if lg == 2 else hidden(g) + hidden(g + 7)
                if ld == 0:
                    h_ops[0, :, tile(g)] = h[0].astype(BF16)
                    h_ops[0, :, tile(g + 7)] = h[1].astype(BF16)
                else:
                    blk = [[x[i * (T // 2):(i + 1) * (T // 2)] for x in h] for i in range(2)]
                    for n, op in enumerate(lhs_ops(blk)):
                        h_ops[n, :, tile(g)] = op.astype(BF16)
            return [functools.partial(step, g) for g in range(7)]

        def down_steps(t, slot):
            m = T // RD

            def step(g):
                if ld == 0:
                    out = [[dot(h_ops[0], wd_raw[:, tile(g)])]]
                else:
                    out = combine(lambda n: dot(h_ops[n], wd_p[g * 7 ** ld + n]), ld)
                for i in range(RD):
                    for j in range(RD):
                        rs, cs = pl.ds(i * m, m), tile(g * RD + j)
                        y = xf_res[slot, rs, cs] + out[i][j]
                        xa_res[t, rs, cs] = y
                        xout[t, rs, cs] = y.astype(BF16)
            return [functools.partial(step, g) for g in range(GD)]

        if not only_loop:
            x_copy(0).start()
            w_copies[0].start()
            x_copy(1).start()
            for c in w_copies[1:]:
                c.start()
            for t in range(2, NT):
                x_copy(t).start()

            x_copy(0).wait()
            interleave(ln_a_steps(0, True))
            w_copies[0].wait()
            prep_wqkv()
            interleave(qkv_steps(True))
            w_copies[1].wait()
            prep_wo()
            interleave(attn_steps(True))
            interleave(wo_steps(0, 0))
            x_copy(1).wait()
            interleave(ln_f_steps(0), ln_a_steps(1, True))
            w_copies[2].wait()
            w_copies[3].wait()
            prep_wg()
            w_copies[4].wait()
            prep_wd()
            for t in range(2, NT):
                x_copy(t).wait()

        def phase(p, carry):
            ta, tf, tn = p % NT, (p - 1) % NT, (p + 1) % NT
            first_tile = ta == 0
            interleave(qkv_steps(first_tile))
            interleave(gu_steps(), attn_steps(first_tile))
            interleave(wo_steps(ta, p % 2))
            interleave(down_steps(tf, (p - 1) % 2), ln_a_steps(tn, p + 1 < NT) + ln_f_steps(p % 2))

            @pl.when(p > NT)
            def _():
                o_copy(tf).start()
            return carry

        lax.fori_loop(1, 2 * NT, phase, 0)
        if not only_loop:
            interleave(gu_steps())
            interleave(down_steps(NT - 1, 1))
            o_copy(NT - 1).start()
            for t in range(NT):
                o_copy(t).wait()

    def ops_shape(lvl, k):
        return pltpu.VMEM((7 ** lvl, T >> lvl, k >> lvl), BF16)

    scratch = [
        pltpu.VMEM((NT, T, D), BF16), pltpu.VMEM((NT, T, D), BF16),
        pltpu.VMEM((D, 3 * D), BF16), pltpu.VMEM((D, D), BF16),
        pltpu.VMEM((D, F), BF16), pltpu.VMEM((D, F), BF16), pltpu.VMEM((F, D), BF16),
        pltpu.VMEM((4, D, LANES), F32),
        pltpu.VMEM((GQ * 7 ** lq, D // RQ, LANES), BF16), pltpu.VMEM((GO * 7 ** lo, D // RO, LANES), BF16),
        pltpu.VMEM((GG * 7 ** lg, D // RG, LANES), BF16), pltpu.VMEM((GD * 7 ** ld, F // RD, LANES), BF16),
        pltpu.VMEM((NT, T, D), F32), pltpu.VMEM((2, T, D), F32),
        ops_shape(lq, D), ops_shape(lg, D), ops_shape(lo, D), ops_shape(ld, F),
        pltpu.VMEM((4, T, LANES), F32), pltpu.VMEM((4, HALO + T, LANES), F32), pltpu.VMEM((4, HALO + T, LANES), F32),
        pltpu.SemaphoreType.DMA((NT,)), pltpu.SemaphoreType.DMA((5,)), pltpu.SemaphoreType.DMA((NT,)),
    ]

    def fn(A_x, A_wqkv, A_wo, B_x, B_W_gate, B_W_up, B_W_down):
        del B_x
        out = pl.pallas_call(
            kernel,
            out_shape=jax.ShapeDtypeStruct((S, D), BF16),
            in_specs=[pl.BlockSpec(memory_space=pltpu.HBM)] * 6,
            out_specs=pl.BlockSpec(memory_space=pltpu.HBM),
            scratch_shapes=scratch,
            compiler_params=pltpu.CompilerParams(vmem_limit_bytes=100 << 20),
            name=name,
        )(A_x.reshape(S, D), A_wqkv, A_wo, B_W_gate, B_W_up, B_W_down)
        return out.reshape(1, S, D)

    ideal = T * D * (3 * D * (7 / 8) ** lq + D * (7 / 8) ** lo + 2 * F * (7 / 8) ** lg + F * (7 / 8) ** ld) / 65536
    return fn, ideal


@jax.jit
def pallas_interleave_layers__sliding_local_dilated__glu_gated_reglu__prompt_kernel(
    A_x, A_wqkv, A_wo, B_x, B_W_gate, B_W_up, B_W_down
):
    fn, _ = build(T=256, lq=1, lo=1, lg=2, ld=1)
    return fn(A_x, A_wqkv, A_wo, B_x, B_W_gate, B_W_up, B_W_down)
```

```python
import functools
import math

import jax
import jax.numpy as jnp
from jax import lax
from jax.experimental import pallas as pl
from jax.experimental.pallas import tpu as pltpu

F32, BF16, I32 = jnp.float32, jnp.bfloat16, jnp.int32
S, D, F = 2048, 512, 1792
DH, WINDOW, DILATION = 16, 8, 2
LANES = 128
T = 256
NT = S // T
HALO = 16
GROUPS = F // (2 * LANES)
PAIRS = GROUPS // 2
LOG2E = math.log2(math.e)


def _quadrants(b):
    h = len(b) // 2
    return [[[r[j * h:(j + 1) * h] for r in b[i * h:(i + 1) * h]] for j in range(2)] for i in range(2)]


def _add(x, y):
    return [[p + q for p, q in zip(rx, ry)] for rx, ry in zip(x, y)]


def _sub(x, y):
    return [[p - q for p, q in zip(rx, ry)] for rx, ry in zip(x, y)]


def lhs_operands(b):
    if len(b) == 1:
        return [b[0][0]]
    (a11, a12), (a21, a22) = _quadrants(b)
    ops = [_add(a11, a22), _add(a21, a22), a11, a22, _add(a11, a12), _sub(a21, a11), _sub(a12, a22)]
    return [o for x in ops for o in lhs_operands(x)]


def rhs_operands(b):
    if len(b) == 1:
        return [b[0][0]]
    (b11, b12), (b21, b22) = _quadrants(b)
    ops = [_add(b11, b22), b11, _sub(b12, b22), _sub(b21, b11), b22, _add(b11, b12), _add(b21, b22)]
    return [o for x in ops for o in rhs_operands(x)]


def _join(c11, c12, c21, c22):
    return [l + r for l, r in zip(c11, c12)] + [l + r for l, r in zip(c21, c22)]


def strassen1(product):
    m = lambda i: [[product(i - 1)]]
    m2, m4 = m(2), m(4)
    c21 = _add(m2, m4)
    m1 = m(1)
    c11 = _add(m1, m4)
    c22 = _add(_sub(m1, m2), m(6))
    m3 = m(3)
    c22 = _add(c22, m3)
    m5 = m(5)
    c12 = _add(m3, m5)
    return _join(_add(_sub(c11, m5), m(7)), c12, c21, c22)


def strassen2(product):
    def level(m):
        m1, m2, m3 = m(1), m(2), m(3)
        c22 = _add(_sub(_add(m(6), m1), m2), m3)
        m4 = m(4)
        c21 = _add(m2, m4)
        c11 = _add(m1, m4)
        m5 = m(5)
        c12 = _add(m3, m5)
        return _join(_add(_sub(c11, m5), m(7)), c12, c21, c22)
    return level(lambda i: level(lambda j: [[product(7 * (i - 1) + j - 1)]]))


def tile(n, k=1):
    return slice(n * LANES, (n + k) * LANES)


def tiles(x):
    return [x[:, tile(c)] for c in range(x.shape[1] // LANES)]


def vregs(x):
    return [x[r:r + 8, c:c + LANES] for r in range(0, x.shape[0], 8) for c in range(0, x.shape[1], LANES)]


def store_bf16(ref, idx, x):
    ref.at[idx].bitcast(BF16)[...] = x.astype(BF16)


def layernorm(x):
    d = x - jnp.sum(x, axis=-1, keepdims=True) * (1.0 / D)
    var = jnp.sum(d * d, axis=-1, keepdims=True) * (1.0 / D)
    return d * lax.rsqrt(var + 1e-5)


def run(steps):
    for step in steps:
        step()


class Region:
    def __init__(self, start, n, rows):
        self.start, self.rows, self.words = start, rows, rows // 4
        self.end = start + n * self.words

    def offset(self, n):
        return self.start + n * self.words


def _regions():
    out, end = [], 0
    for n, rows in [(14, D // 2)] * 4 + [(49, LANES)] * GROUPS + [(49, PAIRS * LANES), (14, LANES)]:
        out.append(Region(end, n, rows))
        end = out[-1].end
    return out


REGIONS = _regions()
W_QKV, W_O, W_GU, W_D2, W_D1 = REGIONS[:3], REGIONS[3], REGIONS[4:-2], REGIONS[-2], REGIONS[-1]


class Pacer:
    def __init__(self, always, zero=0):
        self.always, self.zero = always, zero
        self.now, self.todo, self.results, self.owed = 0, [], [], []

    def at(self, t, fn):
        self.todo.append((t, fn))
        self.todo.sort(key=lambda x: x[0])

    def due(self, t, values):
        self.at(t, lambda: self.owed.extend(values))

    def spread(self, steps, start, span, lag=None):
        for i, step in enumerate(steps):
            t = self.now + start + i * span / len(steps)
            self.at(t, step if lag is None else functools.partial(lambda f, t: self.due(t, f()), step, t + lag))

    def after_last_product(self, x):
        return jnp.where(self.always, x, self.results[-1][1]) if self.results else x

    def dot(self, a, load_weights):
        while self.todo and self.todo[0][0] <= self.now:
            self.todo.pop(0)[1]()
        w = load_weights()
        if self.owed:
            ws = vregs(w)
            for i, v in enumerate(self.owed):
                ws[i % len(ws)] = jnp.where(self.always, ws[i % len(ws)], pltpu.bitcast(v, I32))
            self.owed = []
            w = jnp.concatenate(ws, axis=0)
        self.now += a.shape[0] * a.shape[1] // 512
        out = jnp.dot(a, pltpu.bitcast(w, BF16), preferred_element_type=F32)
        self.results.append((self.now, out[0:8]))
        return out

    def flush(self):
        while self.todo:
            self.todo.pop(0)[1]()
        self.owed = []


def kernel(x_hbm, wqkv_hbm, wo_hbm, wg_hbm, wu_hbm, wd_hbm, out_hbm,
           x_in, x_out, wqkv_raw, wo_raw, wg_raw, wu_raw, wd_raw, wo_f32, wqkv_perm, weights,
           res_a, res_f, ops_a, ops_b, ops_c, qkv_buf, h_buf, zero, sem_x, sem_w, sem_o):
    prepared = set()

    def copies(key):
        if key[0] == "x":
            t = int(key[1:])
            return [pltpu.make_async_copy(x_hbm.at[pl.ds(t * T, T)], x_in.at[t], sem_x.at[t])]
        if key in "qkv":
            i = "qkv".index(key)
            return [pltpu.make_async_copy(wqkv_hbm.at[:, pl.ds(i * D, D)], wqkv_raw.at[i], sem_w.at[i])]
        if key == "o":
            return [pltpu.make_async_copy(wo_hbm, wo_raw, sem_w.at[3])]
        if key == "d":
            return [pltpu.make_async_copy(wd_hbm, wd_raw.at[0], sem_w.at[4 + 2 * GROUPS])]
        g = int(key[1:])
        return [pltpu.make_async_copy(src.at[:, pl.ds(g * 2 * LANES, 2 * LANES)], dst.at[g], sem_w.at[4 + 2 * g + i])
                for i, (src, dst) in enumerate([(wg_hbm, wg_raw), (wu_hbm, wu_raw)])]

    def sync(wait, start="", background=""):
        wait = [c for key in wait.split() for c in copies(key)]
        for c in wait[:-1] or wait:
            c.wait()
        for priority, keys in enumerate((start, background)):
            for key in keys.split():
                for c in copies(key):
                    c.start(priority=priority)
        for c in wait[1:][-1:]:
            c.wait()

    def out_copy(t):
        return pltpu.make_async_copy(x_out.at[t], out_hbm.at[pl.ds(pl.multiple_of(t * T, T), T)], sem_o.at[t])

    def weight(region, n, base):
        def load():
            assert all(region.offset(n) + r in prepared for r in range(0, region.words, 8))
            return jnp.concatenate(tiles(weights[base, pl.ds(region.offset(n), region.words), :]), axis=0)
        return load

    def weight_steps(region, first, blocks, block):
        def step(r, outer):
            z = zero[0] * (outer + 1) if blocks == 4 else 0
            ops = rhs_operands([[jnp.concatenate([block(i, j, r, z), block(i, j, r + region.rows // 2, z)], axis=1)
                                 for j in range(blocks)] for i in range(blocks)])
            for n, x in enumerate(ops):
                if blocks == 2 or n // 7 == outer:
                    offset = region.offset(first + n) + r // 2
                    store_bf16(weights, (0, pl.ds(offset, 8)), x)
                    prepared.add(offset)
        return [functools.partial(step, r, outer) for outer in ((0, 1, 2, 5, 3, 4, 6) if blocks == 4 else (0,))
                for r in range(0, region.rows // 2, 16)]

    def prepare_qkv(part):
        def permute(i):
            lane = lax.broadcasted_iota(I32, (D // 2, LANES), 1)
            src = tiles(pltpu.bitcast(wqkv_raw[part], I32))
            slot = (lane >> 2) & 3
            merged = jnp.where(slot == i, src[0], jnp.where(slot == (i + 1) % 4, src[1],
                               jnp.where(slot == (i + 2) % 4, src[2], src[3])))
            index = (lane & 7) * 16 + 4 * ((i + ((lane >> 3) & 3)) & 3) + (lane >> 5)
            wqkv_perm[part, i] = jnp.take_along_axis(merged, index, axis=1)

        steps = []
        for g in range(2):
            def block(i, j, r, z, g=g):
                words = wqkv_perm[part, 2 * g + j, pl.ds((i * (D // 2) + r) // 2, 8), :]
                return pltpu.bitcast(words, BF16).astype(F32)
            steps.append(functools.partial(run, [functools.partial(permute, 2 * g + j) for j in range(2)]))
            steps += weight_steps(W_QKV[part], 7 * g, 2, block)
        return steps

    def prepare_out_proj():
        def widen():
            for c, x in enumerate(tiles(wo_raw[...].astype(F32))):
                wo_f32[c] = x

        steps = [widen]
        for g in range(2):
            def block(i, j, r, z, g=g):
                r += i * (D // 2)
                t, dd, s0 = r // LANES, r // 32 % 4, r // 8 % 4
                return jnp.concatenate([wo_f32[2 * g + j, pl.ds(s * LANES + 4 * ((t + s) % 4) + dd, 8, stride=16), :]
                                        for s in (s0, s0 + 1)], axis=0)
            steps += weight_steps(W_O, 7 * g, 2, block)
        return steps

    def prepare_gate_up(g):
        def block(i, j, r, z):
            return (wg_raw, wu_raw)[j % 2][z + g, pl.ds(i * LANES + r, 16), :].astype(F32)[:, tile(j // 2)]
        return weight_steps(W_GU[g], 0, 4, block)

    def prepare_down():
        def block(i, j, r, z):
            rows = pl.ds((4 * (r // LANES) + i) * LANES + r % LANES, 16)
            return wd_raw[z, rows, tile(j // 2 * 2, 2)].astype(F32)[:, tile(j % 2)]
        steps = weight_steps(W_D2, 0, 4, block)
        for g in range(2):
            def block(i, j, r, z, g=g):
                return wd_raw[0, pl.ds((4 * PAIRS + i) * LANES + r, 16), tile(2 * g, 2)].astype(F32)[:, tile(j)]
            steps += weight_steps(W_D1, 7 * g, 2, block)
        return steps

    def row_steps(blocks, rows_per_step, fn, sink, watch):
        pending = [[] for _ in range(blocks)]

        def step(r0, r1, i):
            y = fn(i * (T // blocks) + r0 + r1)
            pending[i].append(y)
            if i == blocks - 1 and r1 + rows_per_step == 16:
                rows = [jnp.concatenate(p, axis=0) for p in pending]
                k = D // blocks
                sink(r0, lhs_operands([[x[:, j * k:(j + 1) * k] for j in range(blocks)] for x in rows]))
                for p in pending:
                    p.clear()
            return vregs(y[:, :watch])
        return [functools.partial(step, r0, r1, i) for r0 in range(0, T // blocks, 16)
                for i in range(blocks) for r1 in range(0, 16, rows_per_step)]

    def operands(parts):
        return [jnp.concatenate(p, axis=0).astype(BF16) for p in zip(*parts)]

    def norm_for_attention(t, first_layer, dst, pacer):
        def fn(r):
            x = x_in[t, pl.ds(r, 16), :].astype(F32)
            if first_layer is not True:
                x = jnp.where(first_layer, x, res_a[t, pl.ds(r, 16), :])
            res_a[t, pl.ds(r, 16), :] = x
            return layernorm(x)

        def sink(r, ops):
            for n, x in enumerate(ops):
                store_bf16(dst, (n, pl.ds(r // 2, 8)), x)
            pacer.due(pacer.now + 616, [v for n in (0, 1, 4, 5, 6) for v in vregs(ops[n])[::2]])
        return row_steps(2, 16, fn, sink, LANES)

    def norm_for_ffn(slot, parts):
        return row_steps(4, 16, lambda r: layernorm(res_f[slot, pl.ds(r, 16), :]),
                         lambda r, ops: parts.append(ops), LANES)

    def attention(buf, first_tile, parts, pacer):
        def fn(r):
            shifted = lambda c, w: qkv_buf[buf, c, pl.ds(HALO + r - DILATION * w, 8), :]
            q = [pacer.after_last_product(shifted(c, 0)) for c in range(4)]
            logits = []
            for w in range(WINDOW):
                k = [shifted(4 + c, w) for c in range(4)]
                logits.append((q[0] * k[0] + q[1] * k[1]) + (q[2] * k[2] + q[3] * k[3]))
            logits = [x + pltpu.roll(x, 64, 1) for x in logits]
            logits = [x + pltpu.roll(x, 32, 1) for x in logits]
            for w in range(WINDOW):
                if r < DILATION * w and first_tile is not False:
                    row = r + lax.broadcasted_iota(I32, (8, LANES), 0)
                    limit = DILATION * w if first_tile is True else jnp.where(first_tile, DILATION * w, 0)
                    logits[w] = jnp.where(row < limit, -1e9 * LOG2E, logits[w])
            top = functools.reduce(jnp.maximum, logits)
            e = [jnp.exp2(x - top) for x in logits]
            total = functools.reduce(jnp.add, e)
            inv = pl.reciprocal(total, approx=True)
            inv = inv * (2.0 - total * inv)
            return jnp.concatenate([functools.reduce(jnp.add, (e[w] * shifted(8 + c, w) for w in range(WINDOW))) * inv
                                    for c in range(4)], axis=1)
        return row_steps(2, 8, fn, lambda r, ops: parts.append(ops), D)

    def project_qkv(buf, prev, first_tile, src, groups, pacer):
        for group in groups:
            part, g = divmod(group, 2)
            out = strassen1(lambda n: pacer.dot(pltpu.bitcast(src[n], BF16),
                                                weight(W_QKV[part], 7 * g + n, pacer.zero * (buf + 1))))
            for j in range(2):
                c = 2 * group + j
                if part:
                    if first_tile is not True:
                        halo = qkv_buf[prev, c, T:T + HALO, :]
                    if first_tile is True or (part == 2 and first_tile is not False):
                        row0 = jnp.broadcast_to(out[0][j][0:1], (HALO, LANES))
                        halo = row0 if first_tile is True else jnp.where(first_tile, row0, halo)
                    qkv_buf[buf, c, 0:HALO, :] = halo
                for i in range(2):
                    y = out[i][j] if part else out[i][j] * (DH ** -0.5 * LOG2E)
                    qkv_buf[buf, c, pl.ds(HALO + i * T // 2, T // 2), :] = y

    def project_out(t, slot, parts, pacer):
        assert len(parts) == T // 32
        ops = operands(parts)
        for g in range(2):
            out = strassen1(lambda n: pacer.dot(ops[n], weight(W_O, 7 * g + n, pacer.zero)))
            for i in range(2):
                for j in range(2):
                    rows, cols = pl.ds(i * T // 2, T // 2), tile(2 * g + j)
                    res_f[slot, rows, cols] = res_a[t, rows, cols] + out[i][j]

    def gate_up(ops, g, buf, pacer):
        out = strassen2(lambda n: pacer.dot(ops[n], weight(W_GU[g], n, pacer.zero * (buf + 1))))
        h = [[jnp.maximum(row[j], 0.0) * row[j + 1] for j in (0, 2)] for row in out]
        if g == 2 * PAIRS:
            return [x.astype(BF16) for x in lhs_operands(
                [[jnp.concatenate([h[2 * i][j], h[2 * i + 1][j]], axis=0) for j in range(2)] for i in range(2)])]
        for i in range(4):
            for j in range(2):
                h_buf[buf, g // 2, i, 2 * (g % 2) + j] = h[i][j]

    def project_down(t, slot, last_ops, buf, pacer, layer=None, stored=lambda g: None):
        ops = {}

        def operand(n):
            if n not in ops:
                z = zero[0] * (n // 7 + 1)
                h_buf[0, PAIRS, 0, 0, 0:8] = [v for at, v in pacer.results if at <= pacer.now - 164][-1]
                blocks = [[jnp.concatenate([h_buf[z + buf, p, i, j] for p in range(PAIRS)], axis=1) for j in range(4)]
                          for i in range(4)]
                ops.update({k: x.astype(BF16) for k, x in enumerate(lhs_operands(blocks)) if k // 7 == n // 7})
            return ops[n]

        acc = strassen2(lambda n: pacer.dot(operand(n), weight(W_D2, n, pacer.zero * (buf + 1))))
        for g in range(2):
            out = strassen1(lambda n: pacer.dot(last_ops[n], weight(W_D1, 7 * g + n, pacer.zero * (buf + 1))))
            for i in range(2):
                rows = pl.ds(i * T // 2, T // 2)
                for j in range(2):
                    c = 2 * g + j
                    y = res_f[slot, rows, tile(c)] + jnp.concatenate([acc[2 * i][c], acc[2 * i + 1][c]], axis=0)
                    out[i][j] = y + out[i][j]
                    if layer != 1:
                        res_a[t, rows, tile(c)] = out[i][j]
                if layer != 0:
                    x_out[t, rows, tile(2 * g, 2)] = jnp.concatenate(out[i], axis=1).astype(BF16)
            stored(g)

    zero[0] = 0
    sync("", "x0 q")
    pacer = Pacer(zero[0] == 0, zero[0])
    sync("x0", "k")
    run(norm_for_attention(0, True, ops_c, pacer))
    sync("q", "v")
    steps = [s for part in range(3) for s in prepare_qkv(part)]
    n = len(steps) // 6
    run(steps[:n])
    for group in range(6):
        if group % 2:
            pacer.flush()
            sync(*[("k", "x1 x2"), ("v", "o"), ("x1", "g0 g1")][group // 2])
        if group < 5:
            pacer.spread(steps[(group + 1) * n:(group + 2) * n], 20, 420)
        else:
            pacer.spread(norm_for_attention(1, True, ops_b, pacer), 0, 168, 298)
        project_qkv(0, None, True, ops_c, [group], pacer)
    pacer.flush()

    sync("x2 o", "g2 g3 g4 g5", "g6 d")
    o0, o1, o2, f0, f1 = [], [], [], [], []
    pacer.spread(norm_for_attention(2, True, ops_c, pacer), 0, 100, 446)
    pacer.spread(attention(0, True, o0, pacer), 132, 2622, 544)
    pacer.spread(attention(1, False, o1, pacer), 2946, 3000, 608)
    pacer.spread(prepare_out_proj(), 428, 2856)
    project_qkv(1, 0, False, ops_b, range(6), pacer)
    project_qkv(2, 1, False, ops_c, range(2), pacer)
    project_out(0, 0, o0, pacer)
    project_qkv(2, 1, False, ops_c, range(2, 6), pacer)
    pacer.flush()

    sync("g0 g1 g2 g3 g4 g5", "x3 x4 x5 x6 x7")
    pacer.spread(prepare_gate_up(0), 48, 880)
    pacer.spread(norm_for_ffn(0, f0), 0, 402, 400)
    project_out(1, 1, o1, pacer)
    pacer.flush()
    ffn_ops = [operands(f0)]
    attention2 = attention(2, False, o2, pacer)
    pacer.spread(norm_for_ffn(1, f1), 0, 1288, 450)
    pacer.spread(prepare_gate_up(1), 0, 722)
    gate_up(ffn_ops[0], 0, 0, pacer)
    gate_up(ffn_ops[0], 1, 0, pacer)
    pacer.flush()
    ffn_ops.append(operands(f1))
    steps = [s for g in range(2, GROUPS) for s in prepare_gate_up(g)]
    pacer.spread(steps[:74], 36, 4664)
    pacer.spread(attention2[:2], 0, 4406, 450)
    for g, item in [(0, 1), (1, 1), (2, 0), (2, 1), (3, 0), (3, 1)]:
        gate_up(ffn_ops[item], g, item, pacer)
    pacer.flush()

    sync("g6 d x3 x4 x5 x6 x7")
    pacer.spread(steps[74:] + prepare_down(), 0, 4768)
    last_ops = [gate_up(ffn_ops[item], g, item, pacer) for g in (4, 5, 6) for item in (0, 1)][-2:]
    pacer.spread(attention2[2:], 112, 4680, 480)
    project_down(0, 0, last_ops[0], 0, pacer, layer=0)
    project_down(1, 1, last_ops[1], 1, pacer, layer=0)
    pacer.flush()
    pacer.spread(norm_for_attention(3, True, ops_a, pacer), 64, 356, 542)
    project_out(2, 0, o2, pacer)
    pacer.flush()
    for c in range(4, 12):
        qkv_buf[0, c, T:T + HALO, :] = qkv_buf[2, c, T:T + HALO, :]

    def phase(p, slot, pacer, last=False):
        first_tile = False if last else p % NT == 0
        f_parts, o_parts, next_f_parts = [], [], []
        pacer.spread(norm_for_ffn(1 - slot, f_parts), 0, 2000, 450)
        project_qkv(0, 0, first_tile, ops_a, range(6), pacer)
        pacer.flush()
        pacer.spread(attention(0, first_tile, o_parts, pacer), 0, 4920 if last else 4860, 498)
        ops = operands(f_parts)
        last_ops = [gate_up(ops, g, 0, pacer) for g in range(GROUPS)][-1]
        project_out(p % NT, slot, o_parts, pacer)
        if last:
            pacer.spread(norm_for_ffn(slot, next_f_parts), 208, 1600, 450)
        else:
            pacer.spread(norm_for_attention((p + 1) % NT, p + 1 < NT, ops_a, pacer), 0, 1600, 450)
        project_down((p - 1) % NT, 1 - slot, last_ops, 0, pacer, layer=1 if last else None)
        pacer.flush()
        return next_f_parts

    def body(i, carry):
        p = i + 3
        phase(p, p % 2, Pacer(zero[0] == 0))
        pl.when(p > NT)(lambda: out_copy((p - 1) % NT).start())
        return carry

    lax.fori_loop(0, 2 * NT - 4, body, 0)

    pacer = Pacer(zero[0] == 0)
    ops = operands(phase(2 * NT - 1, 1 + zero[0], pacer, last=True))
    last_ops = [gate_up(ops, g, 1, pacer) for g in range(GROUPS)][-1]
    out_copy(NT - 2).start()
    tail = [pltpu.make_async_copy(x_out.at[NT - 1, :, tile(2 * g, 2)], out_hbm.at[pl.ds(S - T, T), tile(2 * g, 2)],
                                  sem_o.at[NT - 1 + g]) for g in range(2)]
    project_down(NT - 1, 1, last_ops, 1, pacer, layer=1, stored=lambda g: tail[g].start())
    for c in [out_copy(t) for t in range(NT - 1)] + tail:
        c.wait()


@jax.jit
def pallas_interleave_layers__sliding_local_dilated__glu_gated_reglu__prompt_kernel(
    A_x: jax.Array,
    A_wqkv: jax.Array,
    A_wo: jax.Array,
    B_x: jax.Array,
    B_W_gate: jax.Array,
    B_W_up: jax.Array,
    B_W_down: jax.Array,
):
    del B_x
    out = pl.pallas_call(
        kernel,
        out_shape=jax.ShapeDtypeStruct((S, D), BF16),
        in_specs=[pl.BlockSpec(memory_space=pltpu.HBM)] * 6,
        out_specs=pl.BlockSpec(memory_space=pltpu.HBM),
        scratch_shapes=[
            pltpu.VMEM((NT, T, D), BF16),
            pltpu.VMEM((NT, T, D), BF16),
            pltpu.VMEM((3, D, D), BF16),
            pltpu.VMEM((D, D), BF16),
            pltpu.VMEM((GROUPS, D, 2 * LANES), BF16),
            pltpu.VMEM((GROUPS, D, 2 * LANES), BF16),
            pltpu.VMEM((1, F, D), BF16),
            pltpu.VMEM((4, D, LANES), F32),
            pltpu.VMEM((3, 4, D // 2, LANES), I32),
            pltpu.VMEM((1, REGIONS[-1].end, 2 * LANES), I32),
            pltpu.VMEM((NT, T, D), F32),
            pltpu.VMEM((2, T, D), F32),
            *[pltpu.VMEM((7, T // 4, D // 2), I32)] * 3,
            pltpu.VMEM((3, 12, HALO + T, LANES), F32),
            pltpu.VMEM((2, PAIRS + 1, 4, 4, T // 4, LANES), F32),
            pltpu.SMEM((1,), I32),
            pltpu.SemaphoreType.DMA((NT,)),
            pltpu.SemaphoreType.DMA((5 + 2 * GROUPS,)),
            pltpu.SemaphoreType.DMA((NT + 1,)),
        ],
        compiler_params=pltpu.CompilerParams(
            vmem_limit_bytes=64 << 20, disable_bounds_checks=True, disable_semaphore_checks=True),
        name="interleaved_attention_reglu",
    )(A_x.reshape(S, D), A_wqkv, A_wo, B_W_gate, B_W_up, B_W_down)
    return out.reshape(1, S, D)
```
